```python
import jax
import jax.numpy as jnp

def _softmax(x, axis=-1):
    return jax.nn.softmax(x, axis=axis)
def _gelu(x):
    return jax.nn.gelu(x, approximate=True)
def _silu(x):
    return jax.nn.silu(x)
def _sigmoid(x):
    return jax.nn.sigmoid(x)
def _layernorm(x, axis=-1, eps=1e-5):
    m = jnp.mean(x, axis=axis, keepdims=True)
    v = jnp.var(x, axis=axis, keepdims=True)
    return (x - m) / jnp.sqrt(v + eps)
def _scatter_add(tgt, idx, src, axis=0):
    return tgt.at[idx].add(src)
def _segment_sum(src, seg, n):
    return jax.ops.segment_sum(src, seg, n)
class _Rng:
    def __init__(self, key):
        self._k = key
    def _next(self):
        self._k, sub = jax.random.split(self._k)
        return sub
    def normal(self, shape):
        return jax.random.normal(self._next(), shape, dtype=jnp.bfloat16)
    def randint(self, lo, hi, shape):
        return jax.random.randint(self._next(), shape, lo, hi, dtype=jnp.int32)
    def uniform(self, shape, lo=0.0, hi=1.0):
        return jax.random.uniform(self._next(), shape, jnp.bfloat16, lo, hi)
    def permutation(self, n):
        return jax.random.permutation(self._next(), n)


kernel_name = 'gated_mix__mha_block_cached__compressed_kv_cla__decode'

def setup_inputs():
    _rng = _Rng(jax.random.key(int.from_bytes(__import__("os").urandom(4), "little")))
    _w = (lambda a: (lambda t: t.astype(jnp.bfloat16) if jnp.issubdtype(t.dtype, jnp.floating) else t)(jnp.asarray(a)))
    def _A_setup():
        B, Sq, D = 2, 1, 512
        H, Sk, Dh = 32, 8192, 128
        return {
            "x": _w((lambda *s: _rng.normal(s) * 0.05)(B, Sq, D)),
            "k_cache": _w((lambda *s: _rng.normal(s) * 0.05)(B, H, Sk, Dh)),
            "v_cache": _w((lambda *s: _rng.normal(s) * 0.05)(B, H, Sk, Dh)),
            "wq": _w((lambda *s: _rng.normal(s) * 0.05)(D, H * Dh) * (D ** -0.5)),
            "wo": _w((lambda *s: _rng.normal(s) * 0.05)(H * Dh, D) * ((H * Dh) ** -0.5)),
        }
    _A_in = _A_setup()

    def _B_setup():
        B, H, Sq, Sk, D, M = 2, 32, 1, 8192, 128, 512
        Dc = 4 * D
        return {
            "x": _w((lambda *s: _rng.normal(s) * 0.05)(B, Sq, M)),
            "c_kv": _w((lambda *s: _rng.normal(s) * 0.05)(B, Sk, Dc)),
            "w_q": _w((lambda *s: _rng.normal(s) * 0.05)(M, H, D) * (M ** -0.5)),
            "w_uk": _w((lambda *s: _rng.normal(s) * 0.05)(Dc, H, D) * (Dc ** -0.5)),
            "w_uv": _w((lambda *s: _rng.normal(s) * 0.05)(Dc, H, D) * (Dc ** -0.5)),
            "w_o": _w((lambda *s: _rng.normal(s) * 0.05)(H, D, M) * ((H * D) ** -0.5)),
        }
    _B_in = _B_setup()

    return {
        "A_x": _A_in["x"],
        "A_k_cache": _A_in["k_cache"],
        "A_v_cache": _A_in["v_cache"],
        "A_wq": _A_in["wq"],
        "A_wo": _A_in["wo"],
        "B_x": _B_in["x"],
        "B_c_kv": _B_in["c_kv"],
        "B_w_q": _B_in["w_q"],
        "B_w_uk": _B_in["w_uk"],
        "B_w_uv": _B_in["w_uv"],
        "B_w_o": _B_in["w_o"],
        "gate_w": _w((lambda *s: _rng.normal(s) * 0.05)(512)),
    }

def reference(A_x, A_k_cache, A_v_cache, A_wq, A_wo, B_x, B_c_kv, B_w_q, B_w_uk, B_w_uv, B_w_o, gate_w):
    def _A_ref(x, k_cache, v_cache, wq, wo):
        B, Sq, D = x.shape
        H, Dh = 32, 128
        q = (lambda x, *d: x.transpose(*d))((x @ wq).reshape(B, Sq, H, Dh), 0, 2, 1, 3)
        scores = jnp.einsum("bhqd,bhkd->bhqk", q, k_cache) * (Dh ** -0.5)
        p = _softmax(scores, axis=-1)
        o = jnp.einsum("bhqk,bhkd->bhqd", p, v_cache)
        return (lambda x, *d: x.transpose(*d))(o, 0, 2, 1, 3).reshape(B, Sq, H * Dh) @ wo

    def _B_ref(x, c_kv, w_q, w_uk, w_uv, w_o):
        B, Sq, M = x.shape[0], x.shape[1], x.shape[2]
        Sk = c_kv.shape[1]
        H, D = w_q.shape[1], w_q.shape[2]
        q = jnp.einsum("bqm,mhd->bhqd", x, w_q)
        k = jnp.einsum("bkc,chd->bhkd", c_kv, w_uk)
        v = jnp.einsum("bkc,chd->bhkd", c_kv, w_uv)
        scores = jnp.einsum("bhqd,bhkd->bhqk", q, k) * (D ** -0.5)
        off = Sk - Sq
        qi = jnp.arange(Sq)[:, None]
        kj = jnp.arange(Sk)[None, :]
        cmask = kj <= (qi + off)
        scores = jnp.where(cmask[None, None], scores, -1e9)
        p = _softmax(scores, axis=-1)
        ctx = jnp.einsum("bhqk,bhkd->bhqd", p, v)
        return jnp.einsum("bhqd,hdm->bqm", ctx, w_o)

    x = A_x
    g = _sigmoid((x * gate_w).sum(-1, keepdims=True))
    a = _A_ref(x, A_k_cache, A_v_cache, A_wq, A_wo)
    b = _B_ref(x, B_c_kv, B_w_q, B_w_uk, B_w_uv, B_w_o)
    return g * a + (1 - g) * b
```

```python
import jax
import jax.numpy as jnp
import jax.experimental.pallas as pl
import jax.experimental.pallas.tpu as pltpu

_B, _H, _SK, _DH, _D, _DC = 2, 32, 8192, 128, 512, 512

_NW = 8
_NG = _B * _H // 8
_WK = _SK // _NW
_LAG = 3
_NSLOT = 4
_NOCHK = True

_f32 = jnp.float32
_bf16 = jnp.bfloat16


def _dot(a, b):
    return jnp.dot(a, b, preferred_element_type=_f32)


def _dot_t(a, b):
    return jax.lax.dot_general(a, b, (((1,), (1,)), ((), ())), preferred_element_type=_f32)


def _unpack_pair(blk):
    lo = pltpu.bitcast(blk << 16, _f32).astype(_bf16)
    hi = pltpu.bitcast(blk & jnp.int32(-65536), _f32).astype(_bf16)
    return lo, hi


def _fold(x, op):
    parts = [x[:, i:i + 128] for i in range(0, x.shape[1], 128)]
    while len(parts) > 1:
        parts = [op(parts[i], parts[i + 1]) for i in range(0, len(parts), 2)]
    return parts[0]


def _aligned(i, n):
    return i if isinstance(i, int) else pl.multiple_of(i, n)


def _kernel(x_hbm, gw_hbm, k_hbm, v_hbm, wq_hbm, wo_hbm, ckv_hbm, bwq_hbm, bwuk_hbm, bwuv_hbm, bwo_hbm,
            out_ref,
            kv_buf, wq_v, wob_v, ckv_v, bw_v, w32,
            qa_s, qb_s, qlat_s, clat_s, o_s, ctx_s, s_s, mv_s, lv_s, av_s, m_s, l_s, acc_s,
            x_ref, gw_ref, kv_sem, c_sem, w_sem, e_sem, x_sem):

    def start(src, dst, sem, prio):
        pltpu.make_async_copy(src, dst, sem).start(priority=prio)

    def wait_all(dst, sem):
        pltpu.make_async_copy(dst, dst, sem).wait()

    def issue_region(src, first, dst, sem, w, unit):
        half = 64 * unit
        for u in range(8):
            for j8 in range(2):
                for j6 in range(2):
                    for q in range(2):
                        pj = j8 + 2 * q
                        start(src.at[first + pj, :, pl.ds(_aligned(j6 * half + (w * 8 + u) * unit, unit), unit)],
                              dst.at[pj, :, pl.ds((j6 * 8 + u) * unit, unit)], sem, q)

    def issue_kv(src, n):
        slot = n % _NSLOT
        issue_region(src, (n // (2 * _NW)) * 4, kv_buf.at[slot], kv_sem.at[slot], n % _NW, 64)

    def issue_ckv(w):
        issue_region(ckv_hbm, 0, ckv_v.at[w], c_sem.at[w], w, 16)

    def wq_piece(x):
        idx = (slice(None), pl.ds(_aligned((x // 4) * 8, 8), 8), pl.ds(_aligned((x % 4) * 1024, 1024), 1024))
        return wq_hbm.at[idx], wq_v.at[idx], w_sem.at[0]

    def bw_piece(j):
        src = (bwq_hbm, bwuk_hbm, bwuv_hbm)[j]
        def piece(x):
            rows = pl.ds(_aligned(x * 64, 64), 64)
            return src.at[:, rows], bw_v.at[j, :, rows], w_sem.at[1 + j]
        return piece

    def issue_weights(pieces, w):
        for u in range(8):
            for j5 in range(2):
                for j6 in range(2):
                    for q in range(2):
                        start(*pieces[q](j6 * 64 + j5 * 32 + w * 8 + u), q)

    def issue_end(chunks):
        for u in range(8):
            for e in chunks:
                for j6 in range(2):
                    for q, src in enumerate((wo_hbm, bwo_hbm)):
                        start(src.at[:, pl.ds(_aligned(j6 * 1024 + e * 128 + u * 16, 16), 16)],
                              wob_v.at[e, q, :, pl.ds(j6 * 128 + u * 16, 16)], e_sem.at[e], q)

    row8 = jax.lax.broadcasted_iota(jnp.int32, (8, _D), 0)
    row8h = jax.lax.broadcasted_iota(jnp.int32, (8, _DH), 0)
    row8k = jax.lax.broadcasted_iota(jnp.int32, (8, _WK), 0)
    scale = _DH ** -0.5

    def two_rows(r0, r1):
        return jnp.where(row8 == 0, r0, jnp.where(row8 == 1, r1, 0.0))

    def compute_qa(x8):
        def body(c, carry):
            cols = pl.ds(pl.multiple_of(c * 512, 512), 512)
            q = _dot(x8, wq_v[:, :, cols].reshape(_D, 512)) * scale
            for j in range(4):
                for b in range(_B):
                    qa_s[pl.ds(b * _H + 4 * c + j, 1), :] = q[b:b + 1, j * _DH:(j + 1) * _DH]
            return carry
        jax.lax.fori_loop(0, _H // 4, body, 0)

    def to_words(j, lo, hi):
        R = 256
        per_half = w32.shape[0] // (2 * R)
        def cp(blk, c):
            w32[pl.ds(pl.multiple_of(blk * R, R), R), :] = pltpu.bitcast(
                bw_v[j, blk // per_half, pl.ds(pl.multiple_of((blk % per_half) * 2 * R, 2 * R), 2 * R), :], jnp.int32)
            return c
        jax.lax.fori_loop(lo * per_half, hi * per_half, cp, 0)

    def head_pair(i):
        return _unpack_pair(w32[pl.ds(i, _D, stride=_H // 2), :])

    def compute_qb(x8, i0, i1):
        def body(i, c):
            lo, hi = head_pair(i)
            qb_s[2 * i] = _dot(x8, lo)
            qb_s[2 * i + 1] = _dot(x8, hi)
            return c
        jax.lax.fori_loop(i0, i1, body, 0)

    def compute_qlat(i0, i1):
        def body(i, c):
            pair = head_pair(i)
            for j in range(2):
                h = 2 * i + j
                ql = _dot_t(qb_s[h].astype(_bf16), pair[j]) * scale
                for b in range(_B):
                    qlat_s[b, pl.ds(h, 1), :] = ql[b:b + 1, :]
            return c
        jax.lax.fori_loop(i0, i1, body, 0)

    def b_chunk(b, w):
        ck = ckv_v[w, pl.ds(2 * b, 2)].reshape(_WK, _DC)
        s = _dot_t(qlat_s[b].astype(_bf16), ck)
        m_old = m_s[b]
        m_new = jnp.maximum(m_old, jnp.max(s, axis=-1, keepdims=True))
        p = jnp.exp(s - m_new)
        alpha = jnp.exp(m_old - m_new)
        m_s[b] = m_new
        l_s[b] = alpha * l_s[b] + jnp.sum(p, axis=-1, keepdims=True)
        acc_s[b] = alpha * acc_s[b] + _dot(p.astype(_bf16), ck)

    def compute_ctx(i0, i1):
        def body(i, c):
            pair = head_pair(i)
            for j in range(2):
                h = 2 * i + j
                lhs = two_rows(clat_s[0, pl.ds(h, 1), :], clat_s[1, pl.ds(h, 1), :])
                ctx_s[h] = _dot(lhs.astype(_bf16), pair[j])
            return c
        jax.lax.fori_loop(i0, i1, body, 0)

    def k_window(g, w, slot):
        q8 = qa_s[pl.ds(pl.multiple_of(g * 8, 8), 8), :].astype(_bf16)
        s = None
        for j in range(8):
            sj = _dot_t(q8, kv_buf[slot, j // 2, j % 2])
            s = sj if s is None else jnp.where(row8k == j, sj, s)
        s_s[:, pl.ds(pl.multiple_of(w * _WK, _WK), _WK)] = s
        mv_s[...] = jnp.maximum(mv_s[...], _fold(s, jnp.maximum))

    def v_window(w, slot):
        m = jnp.max(mv_s[...], axis=-1, keepdims=True)
        p = jnp.exp(s_s[:, pl.ds(pl.multiple_of(w * _WK, _WK), _WK)] - m)
        lv_s[...] += _fold(p, jnp.add)
        p = p.astype(_bf16)
        o = None
        for j in range(8):
            oj = _dot(p, kv_buf[slot, j // 2, j % 2])
            o = oj if o is None else jnp.where(row8h == j, oj, o)
        av_s[...] += o

    def reset_group():
        mv_s[...] = jnp.full_like(mv_s, -jnp.inf)
        lv_s[...] = jnp.zeros_like(lv_s)
        av_s[...] = jnp.zeros_like(av_s)

    def finish_group(g):
        o = av_s[...] / jnp.sum(lv_s[...], axis=-1, keepdims=True)
        for j in range(8):
            o_s[(g % 4) * 8 + j, pl.ds(g // 4, 1), :] = o[j:j + 1, :]

    first = (wq_piece, bw_piece(0))
    second = (bw_piece(1), bw_piece(2))
    issue_weights(first, 0)
    cx = pltpu.make_async_copy(x_hbm, x_ref, x_sem.at[0])
    cg = pltpu.make_async_copy(gw_hbm, gw_ref, x_sem.at[1])
    cx.start()
    cg.start()
    o_s[...] = jnp.zeros_like(o_s)
    m_s[...] = jnp.full_like(m_s, -jnp.inf)
    l_s[...] = jnp.zeros_like(l_s)
    acc_s[...] = jnp.zeros_like(acc_s)
    reset_group()
    jax.lax.fori_loop(1, 4, lambda w, c: (issue_weights(first, w), c)[1], 0)
    cx.wait()
    cg.wait()
    xf = x_ref[...].astype(_f32)
    x8f = two_rows(xf[0:1], xf[1:2])
    x8 = x8f.astype(_bf16)
    gate = jax.nn.sigmoid(jnp.sum(x8f * gw_ref[...].astype(_f32).reshape(1, _D), axis=-1, keepdims=True))

    def phase1(w, c):
        issue_weights(second, w)

        @pl.when(w == 0)
        def _():
            wait_all(wq_v, w_sem.at[0])
            compute_qa(x8)

        @pl.when(w == 1)
        def _():
            wait_all(bw_v.at[0], w_sem.at[1])
            to_words(0, 0, 2)

        @pl.when(w >= 2)
        def _():
            compute_qb(x8, (w - 2) * 8, (w - 1) * 8)
        return c
    jax.lax.fori_loop(0, 4, phase1, 0)

    def phase2(t, c):
        @pl.when(t < _NW)
        def _():
            issue_ckv(jnp.minimum(t, _NW - 1))

        @pl.when(t >= _NW)
        def _():
            issue_kv(k_hbm, jnp.maximum(t - _NW, 0))

        @pl.when(t == 0)
        def _():
            wait_all(bw_v.at[1], w_sem.at[2])
            to_words(1, 0, 2)

        @pl.when((t == 1) | (t == 2))
        def _():
            compute_qlat((t - 1) * 8, t * 8)

        @pl.when(t >= _LAG)
        def _():
            w = jnp.maximum(t - _LAG, 0)
            wait_all(ckv_v.at[w], c_sem.at[w])
            jax.lax.fori_loop(0, _B, lambda b, c: (b_chunk(b, w), c)[1], 0)
        return c
    jax.lax.fori_loop(0, _NW + _LAG, phase2, 0)
    clat_s[...] = acc_s[...] / l_s[...]
    wait_all(bw_v.at[2], w_sem.at[3])

    NKV = _NG * 2 * _NW

    def phase3(n, c):
        nxt = n + _LAG
        nxt_is_v = (nxt // _NW) % 2 == 1

        @pl.when((nxt < NKV) & jnp.logical_not(nxt_is_v))
        def _():
            issue_kv(k_hbm, jnp.minimum(nxt, NKV - 1))

        @pl.when((nxt < NKV) & nxt_is_v)
        def _():
            issue_kv(v_hbm, jnp.minimum(nxt, NKV - 1))

        @pl.when(nxt >= NKV)
        def _():
            e = jnp.maximum(nxt - NKV, 0)
            issue_end((2 * e, 2 * e + 1))

        slot = n % _NSLOT
        g = n // (2 * _NW)
        w = n % _NW
        is_v = (n // _NW) % 2 == 1
        wait_all(kv_buf.at[slot], kv_sem.at[slot])

        @pl.when(jnp.logical_not(is_v))
        def _():
            k_window(g, w, slot)

        @pl.when(is_v)
        def _():
            v_window(w, slot)

        @pl.when(n % (2 * _NW) == 2 * _NW - 1)
        def _():
            finish_group(g)
            reset_group()

        @pl.when(n < 2)
        def _():
            to_words(2, n, n + 1)

        @pl.when((n >= 2) & (n < 6))
        def _():
            compute_ctx((n - 2) * 4, (n - 1) * 4)
        return c
    jax.lax.fori_loop(0, NKV, phase3, 0)

    for e in range(2 * _LAG, 8):
        issue_end((e,))

    def phase4(e, acc):
        wait_all(wob_v.at[e], e_sem.at[e])
        out = []
        for q, src in enumerate((o_s, ctx_s)):
            t = acc[q]
            for j in range(4):
                t = t + _dot(src[e + 8 * j].astype(_bf16), wob_v[e, q, j // 2, pl.ds((j % 2) * _DH, _DH), :])
            out.append(t)
        return tuple(out)
    zero = jnp.zeros((8, _D), _f32)
    out_a, out_b = jax.lax.fori_loop(0, 8, phase4, (zero, zero))
    res = gate * out_a + (1.0 - gate) * out_b
    out_ref[...] = res[0:2, :].astype(_bf16)


@jax.jit
def pallas_gated_mix__mha_block_cached__compressed_kv_cla__decode_kernel(
    A_x: jax.Array,
    A_k_cache: jax.Array,
    A_v_cache: jax.Array,
    A_wq: jax.Array,
    A_wo: jax.Array,
    B_x: jax.Array,
    B_c_kv: jax.Array,
    B_w_q: jax.Array,
    B_w_uk: jax.Array,
    B_w_uv: jax.Array,
    B_w_o: jax.Array,
    gate_w: jax.Array,
):
    del B_x
    k4 = A_k_cache.reshape(_B * _H // 2, 2, _SK, _DH)
    v4 = A_v_cache.reshape(_B * _H // 2, 2, _SK, _DH)
    ckv = B_c_kv.reshape(4, 2, _SK // 4, _DC)
    wq = A_wq.reshape(2, _D // 2, _H * _DH)
    bwq = B_w_q.reshape(2, _D * _H // 2, _DH)
    bwuk = B_w_uk.reshape(2, _DC * _H // 2, _DH)
    bwuv = B_w_uv.reshape(2, _DC * _H // 2, _DH)
    wo = A_wo.reshape(2, _H * _DH // 2, _D)
    bwo = B_w_o.reshape(2, _H * _DH // 2, _D)
    x2 = A_x.reshape(_B, _D)

    hbm = pl.BlockSpec(memory_space=pl.ANY)
    vmem = pl.BlockSpec(memory_space=pltpu.VMEM)
    V = pltpu.VMEM
    scratch = [
        V((_NSLOT, 4, 2, _WK, _DH), _bf16),
        V((2, _D // 2, _H * _DH), _bf16),
        V((8, 2, 2, 2 * _DH, _D), _bf16),
        V((_NW, 4, 2, _WK // 4, _DC), _bf16),
        V((3, 2, _D * _H // 2, _DH), _bf16),
        V((_D * _H // 2, _DH), jnp.int32),
        V((_B * _H, _DH), _f32),
        V((_H, 8, _DH), _f32),
        V((_B, _H, _DC), _f32),
        V((_B, _H, _DC), _f32),
        V((_H, 8, _DH), _f32),
        V((_H, 8, _DH), _f32),
        V((8, _SK), _f32),
        V((8, _DH), _f32),
        V((8, _DH), _f32),
        V((8, _DH), _f32),
        V((_B, _H, 1), _f32),
        V((_B, _H, 1), _f32),
        V((_B, _H, _DC), _f32),
        V((_B, _D), _bf16),
        V((_D,), _bf16),
        pltpu.SemaphoreType.DMA((_NSLOT,)),
        pltpu.SemaphoreType.DMA((_NW,)),
        pltpu.SemaphoreType.DMA((4,)),
        pltpu.SemaphoreType.DMA((8,)),
        pltpu.SemaphoreType.DMA((2,)),
    ]
    out = pl.pallas_call(
        _kernel,
        out_shape=jax.ShapeDtypeStruct((_B, _D), _bf16),
        in_specs=[hbm] * 11,
        out_specs=vmem,
        scratch_shapes=scratch,
        compiler_params=pltpu.CompilerParams(vmem_limit_bytes=100 * 1024 * 1024, disable_bounds_checks=_NOCHK),
    )(x2, gate_w, k4, v4, wq, wo, ckv, bwq, bwuk, bwuv, bwo)
    return out.reshape(_B, 1, _D)
```

```python
import jax
import jax.numpy as jnp
import jax.experimental.pallas as pl
import jax.experimental.pallas.tpu as pltpu

_B, _H, _SK, _DH, _D, _DC = 2, 32, 8192, 128, 512, 512

_NW = 8
_NG = _B * _H // 8
_WK = _SK // _NW
_LAG = 3
_NSLOT = _LAG + 1

_f32 = jnp.float32
_bf16 = jnp.bfloat16


def _dot(a, b):
    return jnp.dot(a, b, preferred_element_type=_f32)


def _dot_t(a, b):
    return jax.lax.dot_general(a, b, (((1,), (1,)), ((), ())), preferred_element_type=_f32)


def _unpack_pair(blk):
    lo = pltpu.bitcast(blk << 16, _f32).astype(_bf16)
    hi = pltpu.bitcast(blk & jnp.int32(-65536), _f32).astype(_bf16)
    return lo, hi


def _fold(x, op):
    parts = [x[:, i:i + 128] for i in range(0, x.shape[1], 128)]
    while len(parts) > 1:
        parts = [op(parts[i], parts[i + 1]) for i in range(0, len(parts), 2)]
    return parts[0]


def _ds(first, size):
    return pl.ds(first if isinstance(first, int) else pl.multiple_of(first, size), size)


def _loop(lo, hi, body):
    jax.lax.fori_loop(lo, hi, lambda i, c: (body(i), c)[1], 0)


def _start(src, dst, sem, prio):
    pltpu.make_async_copy(src, dst, sem).start(priority=prio)


def _wait_all(dst, sem):
    pltpu.make_async_copy(dst, dst, sem).wait()


def _kernel(x_hbm, gw_hbm, k_hbm, v_hbm, wq_hbm, wo_hbm, ckv_hbm, bwq_hbm, bwuk_hbm, bwuv_hbm, bwo_hbm,
            out_ref,
            kv_buf, wq_v, wob_v, ckv_v, bw_v, w32,
            qa_s, qb_s, qlat_s, clat_s, o_s, ctx_s, s_s, mv_s, lv_s, av_s, m_s, l_s, acc_s, gate_s,
            x_ref, gw_ref):

    row8 = jax.lax.broadcasted_iota(jnp.int32, (8, _D), 0)
    row8h = jax.lax.broadcasted_iota(jnp.int32, (8, _DH), 0)
    row8k = jax.lax.broadcasted_iota(jnp.int32, (8, _WK), 0)
    scale = _DH ** -0.5

    def two_rows(r0, r1):
        return jnp.where(row8 == 0, r0, jnp.where(row8 == 1, r1, 0.0))

    def compute_qa(x8):
        def body(c):
            q = _dot(x8, wq_v[:, :, _ds(c * 512, 512)].reshape(_D, 512)) * scale
            for j in range(4):
                for b in range(_B):
                    qa_s[pl.ds(b * _H + 4 * c + j, 1), :] = q[b:b + 1, j * _DH:(j + 1) * _DH]
        _loop(0, _H // 4, body)

    def to_words(j, lo, hi):
        R = 256
        per_half = w32.shape[0] // (2 * R)
        def body(i):
            w32[_ds(i * R, R), :] = pltpu.bitcast(
                bw_v[j, i // per_half, _ds((i % per_half) * 2 * R, 2 * R), :], jnp.int32)
        _loop(lo * per_half, hi * per_half, body)

    def head_pair(i):
        return _unpack_pair(w32[pl.ds(i, _D, stride=_H // 2), :])

    def compute_qb(x8, i0, i1):
        def body(i):
            lo, hi = head_pair(i)
            qb_s[2 * i] = _dot(x8, lo)
            qb_s[2 * i + 1] = _dot(x8, hi)
        _loop(i0, i1, body)

    def compute_qlat(i0, i1):
        def body(i):
            pair = head_pair(i)
            for j in range(2):
                h = 2 * i + j
                ql = _dot_t(qb_s[h].astype(_bf16), pair[j]) * scale
                for b in range(_B):
                    qlat_s[b, pl.ds(h, 1), :] = ql[b:b + 1, :]
        _loop(i0, i1, body)

    def b_chunk(b, w):
        ck = ckv_v[w, pl.ds(2 * b, 2)].reshape(_WK, _DC)
        s = _dot_t(qlat_s[b].astype(_bf16), ck)
        m_old = m_s[b]
        m_new = jnp.maximum(m_old, jnp.max(s, axis=-1, keepdims=True))
        p = jnp.exp(s - m_new)
        alpha = jnp.exp(m_old - m_new)
        m_s[b] = m_new
        l_s[b] = alpha * l_s[b] + jnp.sum(p, axis=-1, keepdims=True)
        acc_s[b] = alpha * acc_s[b] + _dot(p.astype(_bf16), ck)

    def compute_ctx(i0, i1):
        def body(i):
            pair = head_pair(i)
            for j in range(2):
                h = 2 * i + j
                lhs = two_rows(clat_s[0, pl.ds(h, 1), :], clat_s[1, pl.ds(h, 1), :])
                ctx_s[h] = _dot(lhs.astype(_bf16), pair[j])
        _loop(i0, i1, body)

    def k_window(g, w, slot):
        q8 = qa_s[_ds(g * 8, 8), :].astype(_bf16)
        s = None
        for j in range(8):
            sj = _dot_t(q8, kv_buf[slot, j // 2, j % 2])
            s = sj if s is None else jnp.where(row8k == j, sj, s)
        s_s[:, _ds(w * _WK, _WK)] = s
        mv_s[...] = jnp.maximum(mv_s[...], _fold(s, jnp.maximum))

    def v_window(w, slot):
        m = jnp.max(mv_s[...], axis=-1, keepdims=True)
        p = jnp.exp(s_s[:, _ds(w * _WK, _WK)] - m)
        lv_s[...] += _fold(p, jnp.add)
        p = p.astype(_bf16)
        o = None
        for j in range(8):
            oj = _dot(p, kv_buf[slot, j // 2, j % 2])
            o = oj if o is None else jnp.where(row8h == j, oj, o)
        av_s[...] += o

    def reset_group():
        mv_s[...] = jnp.full_like(mv_s, -jnp.inf)
        lv_s[...] = jnp.zeros_like(lv_s)
        av_s[...] = jnp.zeros_like(av_s)

    def finish_group(g):
        o = av_s[...] / jnp.sum(lv_s[...], axis=-1, keepdims=True)
        for j in range(8):
            o_s[(g % 4) * 8 + j, pl.ds(g // 4, 1), :] = o[j:j + 1, :]

    def gated(q, h):
        gate = gate_s[...]
        return ((o_s[h] * gate) if q == 0 else (ctx_s[h] * (1.0 - gate))).astype(_bf16)

    def project(lhs, e, q, j6, j7):
        return _dot(lhs, wob_v[e, q, j7, pl.ds(j6 * _DH, _DH), :])

    def run(kv_sem, c_sem, w_sem, e_sem, x_sem):
        def issue_region(src, first, dst, sem, w, unit):
            for u in range(8):
                for j8 in range(2):
                    for j6 in range(2):
                        for q in range(2):
                            pj = j8 + 2 * q
                            _start(src.at[first + pj, :, _ds((j6 * 64 + w * 8 + u) * unit, unit)],
                                   dst.at[pj, :, pl.ds((j6 * 8 + u) * unit, unit)], sem, q)

        def issue_kv(src, n):
            slot = n % _NSLOT
            issue_region(src, (n // (2 * _NW)) * 4, kv_buf.at[slot], kv_sem.at[slot], n % _NW, 64)

        def wq_piece(x):
            idx = (slice(None), _ds((x // 4) * 8, 8), _ds((x % 4) * 1024, 1024))
            return wq_hbm.at[idx], wq_v.at[idx], w_sem.at[0]

        def bw_piece(j):
            src = (bwq_hbm, bwuk_hbm, bwuv_hbm)[j]
            return lambda x: (src.at[:, _ds(x * 64, 64)], bw_v.at[j, :, _ds(x * 64, 64)], w_sem.at[1 + j])

        def issue_weights(pieces, w):
            for u in range(8):
                for j5 in range(2):
                    for j6 in range(2):
                        for q in range(2):
                            _start(*pieces[q](j6 * 64 + j5 * 32 + w * 8 + u), q)

        def end_piece(e, q, j6, u):
            return ((wo_hbm, bwo_hbm)[q].at[:, _ds(j6 * 1024 + e * 128 + u * 16, 16)],
                    wob_v.at[e, q, :, pl.ds(j6 * 128 + u * 16, 16)])

        def issue_end(chunks):
            for u in range(8):
                for e in chunks:
                    for j6 in range(2):
                        for q in range(2):
                            _start(*end_piece(e, q, j6, u), e_sem.at[e], q)

        first = (wq_piece, bw_piece(0))
        second = (bw_piece(1), bw_piece(2))
        issue_weights(first, 0)
        cx = pltpu.make_async_copy(x_hbm, x_ref, x_sem.at[0])
        cg = pltpu.make_async_copy(gw_hbm, gw_ref, x_sem.at[1])
        cx.start()
        cg.start()
        o_s[...] = jnp.zeros_like(o_s)
        m_s[...] = jnp.full_like(m_s, -jnp.inf)
        l_s[...] = jnp.zeros_like(l_s)
        acc_s[...] = jnp.zeros_like(acc_s)
        reset_group()
        _loop(1, 4, lambda w: issue_weights(first, w))
        cx.wait()
        cg.wait()
        xf = x_ref[...].astype(_f32)
        x8f = two_rows(xf[0:1], xf[1:2])
        x8 = x8f.astype(_bf16)
        gate = jax.nn.sigmoid(jnp.sum(x8f * gw_ref[...].astype(_f32).reshape(1, _D), axis=-1, keepdims=True))
        gate_s[...] = jnp.broadcast_to(gate, (8, _DH))

        def phase1(w):
            issue_weights(second, w)

            @pl.when(w == 0)
            def _():
                _wait_all(wq_v, w_sem.at[0])
                compute_qa(x8)

            @pl.when(w == 1)
            def _():
                _wait_all(bw_v.at[0], w_sem.at[1])
                to_words(0, 0, 2)

            @pl.when(w >= 2)
            def _():
                compute_qb(x8, (w - 2) * 8, (w - 1) * 8)
        _loop(0, 4, phase1)

        def phase2(t):
            @pl.when(t < _NW)
            def _():
                w = jnp.minimum(t, _NW - 1)
                issue_region(ckv_hbm, 0, ckv_v.at[w], c_sem.at[w], w, 16)

            @pl.when(t >= _NW)
            def _():
                issue_kv(k_hbm, jnp.maximum(t - _NW, 0))

            @pl.when(t == 0)
            def _():
                _wait_all(bw_v.at[1], w_sem.at[2])
                to_words(1, 0, 2)

            @pl.when((t == 1) | (t == 2))
            def _():
                compute_qlat((t - 1) * 8, t * 8)

            @pl.when(t >= _LAG)
            def _():
                w = jnp.maximum(t - _LAG, 0)
                _wait_all(ckv_v.at[w], c_sem.at[w])
                _loop(0, _B, lambda b: b_chunk(b, w))
        _loop(0, _NW + _LAG, phase2)
        clat_s[...] = acc_s[...] / l_s[...]
        _wait_all(bw_v.at[2], w_sem.at[3])

        nkv = _NG * 2 * _NW

        def phase3(n):
            nxt = n + _LAG
            nxt_is_v = (nxt // _NW) % 2 == 1

            @pl.when((nxt < nkv) & jnp.logical_not(nxt_is_v))
            def _():
                issue_kv(k_hbm, jnp.minimum(nxt, nkv - 1))

            @pl.when((nxt < nkv) & nxt_is_v)
            def _():
                issue_kv(v_hbm, jnp.minimum(nxt, nkv - 1))

            @pl.when(nxt >= nkv)
            def _():
                e = jnp.maximum(nxt - nkv, 0)
                issue_end((e, e + 4))

            slot = n % _NSLOT
            g = n // (2 * _NW)
            w = n % _NW
            is_v = (n // _NW) % 2 == 1
            _wait_all(kv_buf.at[slot], kv_sem.at[slot])

            @pl.when(jnp.logical_not(is_v))
            def _():
                k_window(g, w, slot)

            @pl.when(is_v)
            def _():
                v_window(w, slot)

            @pl.when(n % (2 * _NW) == 2 * _NW - 1)
            def _():
                finish_group(g)
                reset_group()

            @pl.when(n < 2)
            def _():
                to_words(2, n, n + 1)

            @pl.when((n >= 2) & (n < 6))
            def _():
                compute_ctx((n - 2) * 4, (n - 1) * 4)
        _loop(0, nkv, phase3)


        parts = (((0, 0), (1, 0)), ((0, 1),), ((1, 1),))
        views = (wob_v.at[7, :, :, pl.ds(0, _DH)], wob_v.at[7, 0, :, pl.ds(_DH, _DH)],
                 wob_v.at[7, 1, :, pl.ds(_DH, _DH)])
        issue_end((3,))
        for i, part in enumerate(parts):
            for u in range(8):
                for k, (q, j6) in enumerate(part):
                    _start(*end_piece(7, q, j6, u), e_sem.at[7 + i], (u * len(part) + k) % 2)

        def phase4(i, acc):
            e = i // 2 + (i % 2) * 4
            _wait_all(wob_v.at[e], e_sem.at[e])
            for q in range(2):
                for j in range(4):
                    acc = acc + project(gated(q, e + 8 * j), e, q, j % 2, j // 2)
            return acc
        res = jax.lax.fori_loop(0, 7, phase4, jnp.zeros((8, _D), _f32))
        for i, part in enumerate(parts):
            blocks = [(q, j6, j7) for q, j6 in part for j7 in range(2)]
            left = [gated(q, 7 + 8 * j6 + 16 * j7) for q, j6, j7 in blocks]
            _wait_all(views[i], e_sem.at[7 + i])
            for blk, lhs in zip(blocks, left):
                res = res + project(lhs, 7, *blk)
        out_ref[...] = res[0:2, :].astype(_bf16)

    dma = pltpu.SemaphoreType.DMA
    pl.run_scoped(run, dma((_NSLOT,)), dma((_NW,)), dma((4,)), dma((10,)), dma((2,)))


@jax.jit
def pallas_gated_mix__mha_block_cached__compressed_kv_cla__decode_kernel(
    A_x: jax.Array,
    A_k_cache: jax.Array,
    A_v_cache: jax.Array,
    A_wq: jax.Array,
    A_wo: jax.Array,
    B_x: jax.Array,
    B_c_kv: jax.Array,
    B_w_q: jax.Array,
    B_w_uk: jax.Array,
    B_w_uv: jax.Array,
    B_w_o: jax.Array,
    gate_w: jax.Array,
):
    del B_x
    k4 = A_k_cache.reshape(_B * _H // 2, 2, _SK, _DH)
    v4 = A_v_cache.reshape(_B * _H // 2, 2, _SK, _DH)
    ckv = B_c_kv.reshape(4, 2, _SK // 4, _DC)
    wq = A_wq.reshape(2, _D // 2, _H * _DH)
    bwq = B_w_q.reshape(2, _D * _H // 2, _DH)
    bwuk = B_w_uk.reshape(2, _DC * _H // 2, _DH)
    bwuv = B_w_uv.reshape(2, _DC * _H // 2, _DH)
    wo = A_wo.reshape(2, _H * _DH // 2, _D)
    bwo = B_w_o.reshape(2, _H * _DH // 2, _D)
    x2 = A_x.reshape(_B, _D)

    hbm = pl.BlockSpec(memory_space=pl.ANY)
    vmem = pl.BlockSpec(memory_space=pltpu.VMEM)
    V = pltpu.VMEM
    scratch = [
        V((_NSLOT, 4, 2, _WK, _DH), _bf16),
        V((2, _D // 2, _H * _DH), _bf16),
        V((8, 2, 2, 2 * _DH, _D), _bf16),
        V((_NW, 4, 2, _WK // 4, _DC), _bf16),
        V((3, 2, _D * _H // 2, _DH), _bf16),
        V((_D * _H // 2, _DH), jnp.int32),
        V((_B * _H, _DH), _f32),
        V((_H, 8, _DH), _f32),
        V((_B, _H, _DC), _f32),
        V((_B, _H, _DC), _f32),
        V((_H, 8, _DH), _f32),
        V((_H, 8, _DH), _f32),
        V((8, _SK), _f32),
        V((8, _DH), _f32),
        V((8, _DH), _f32),
        V((8, _DH), _f32),
        V((_B, _H, 1), _f32),
        V((_B, _H, 1), _f32),
        V((_B, _H, _DC), _f32),
        V((8, _DH), _f32),
        V((_B, _D), _bf16),
        V((_D,), _bf16),
    ]
    out = pl.pallas_call(
        _kernel,
        out_shape=jax.ShapeDtypeStruct((_B, _D), _bf16),
        in_specs=[hbm] * 11,
        out_specs=vmem,
        scratch_shapes=scratch,
        compiler_params=pltpu.CompilerParams(vmem_limit_bytes=100 * 1024 * 1024),
    )(x2, gate_w, k4, v4, wq, wo, ckv, bwq, bwuk, bwuv, bwo)
    return out.reshape(_B, 1, _D)
```

```python
import jax
import jax.numpy as jnp
import jax.experimental.pallas as pl
import jax.experimental.pallas.tpu as pltpu

_B, _H, _SK, _DH, _D, _DC = 2, 32, 8192, 128, 512, 512

_NW = 8
_NG = _B * _H // 8
_WK = _SK // _NW
_LAG = 3
_NSLOT = _LAG + 1
_ROT = 1

_PLAN = (((0, 0), (4, 0)), ((0, 1), (4, 1)), ((2, 0), (6, 0)), ((2, 1), (6, 1)))
_PLAN_WRAP = (((0, 0), (7, None)), ((0, 1), (4, 1)), ((2, 0), (4, 0)), ((2, 1), (6, None)))
_PLAN_CKV = (((1, 0), (0, None)), ((1, 1), (5, 1)), ((3, 0), (5, 0)), ((3, 1), (7, None)))

_f32 = jnp.float32
_bf16 = jnp.bfloat16


def _dot(a, b):
    return jnp.dot(a, b, preferred_element_type=_f32)


def _dot_t(a, b):
    return jax.lax.dot_general(a, b, (((1,), (1,)), ((), ())), preferred_element_type=_f32)


def _unpack_pair(blk):
    lo = pltpu.bitcast(blk << 16, _f32).astype(_bf16)
    hi = pltpu.bitcast(blk & jnp.int32(-65536), _f32).astype(_bf16)
    return lo, hi


def _fold(x, op):
    parts = [x[:, i:i + 128] for i in range(0, x.shape[1], 128)]
    while len(parts) > 1:
        parts = [op(parts[i], parts[i + 1]) for i in range(0, len(parts), 2)]
    return parts[0]


def _ds(first, size):
    return pl.ds(first if isinstance(first, int) else pl.multiple_of(first, size), size)


def _loop(lo, hi, body):
    jax.lax.fori_loop(lo, hi, lambda i, c: (body(i), c)[1], 0)


def _start(src, dst, sem, prio):
    pltpu.make_async_copy(src, dst, sem).start(priority=prio)


def _wait_all(dst, sem):
    pltpu.make_async_copy(dst, dst, sem).wait()


def _kernel(x_hbm, gw_hbm, k_hbm, v_hbm, wq_hbm, wo_hbm, ckv_hbm, bwq_hbm, bwuk_hbm, bwuv_hbm, bwo_hbm,
            out_ref,
            kv_buf, wq_v, wob_v, ckv_v, bw_v, w32,
            x_s, gate_s, qa_s, qb_s, qlat_s, o_s, ctx_s, s_s, mv_s, lv_s, av_s, m_s, l_s, acc_s,
            x_ref, gw_ref):
    row8 = jax.lax.broadcasted_iota(jnp.int32, (8, _D), 0)
    row8h = jax.lax.broadcasted_iota(jnp.int32, (8, _DH), 0)
    row8k = jax.lax.broadcasted_iota(jnp.int32, (8, _WK), 0)
    scale = _DH ** -0.5

    def two_rows(r0, r1):
        return jnp.where(row8 == 0, r0, jnp.where(row8 == 1, r1, 0.0))

    def compute_qa():
        def body(c):
            q = _dot(x_s[...].astype(_bf16), wq_v[:, :, _ds(c * 512, 512)].reshape(_D, 512)) * scale
            for j in range(4):
                for b in range(_B):
                    row = (b * _H + 4 * c + j + _B * _H - _ROT) % (_B * _H)
                    qa_s[pl.ds(row, 1), :] = q[b:b + 1, j * _DH:(j + 1) * _DH]
        _loop(0, _H // 4, body)

    def k_window(g, w, slot):
        q8 = qa_s[_ds(g * 8, 8), :].astype(_bf16)
        s = None
        for j in range(8):
            sj = _dot_t(q8, kv_buf[slot, j].reshape(_WK, _DH))
            s = sj if s is None else jnp.where(row8k == j, sj, s)
        s_s[:, _ds(w * _WK, _WK)] = s
        mv_s[...] = jnp.maximum(mv_s[...], _fold(s, jnp.maximum))

    def v_window(w, slot):
        m = jnp.max(mv_s[...], axis=-1, keepdims=True)
        p = jnp.exp(s_s[:, _ds(w * _WK, _WK)] - m)
        lv_s[...] += _fold(p, jnp.add)
        p = p.astype(_bf16)
        o = None
        for j in range(8):
            oj = _dot(p, kv_buf[slot, j].reshape(_WK, _DH))
            o = oj if o is None else jnp.where(row8h == j, oj, o)
        av_s[...] += o

    def reset_group():
        mv_s[...] = jnp.full_like(mv_s, -jnp.inf)
        lv_s[...] = jnp.zeros_like(lv_s)
        av_s[...] = jnp.zeros_like(av_s)

    def finish_group(g):
        o = av_s[...] / jnp.sum(lv_s[...], axis=-1, keepdims=True)
        for j in range(8):
            f = (g * 8 + j + _ROT) % (_B * _H)
            o_s[f % _H, pl.ds(f // _H, 1), :] = o[j:j + 1, :]

    def to_words(j, half):
        R = 256
        n = w32.shape[0] // (2 * R)
        def body(i):
            w32[_ds((half * n + i) * R, R), :] = pltpu.bitcast(bw_v[j, half, _ds(i * 2 * R, 2 * R), :], jnp.int32)
        _loop(0, n, body)

    def head_pair(i):
        return _unpack_pair(w32[pl.ds(i, _D, stride=_H // 2), :])

    def compute_qb(part):
        def body(i):
            for j, w in enumerate(head_pair(i)):
                qb_s[2 * i + j] = _dot(x_s[...].astype(_bf16), w)
        _loop(part * 4, part * 4 + 4, body)

    def compute_qlat(part):
        def body(i):
            for j, w in enumerate(head_pair(i)):
                h = 2 * i + j
                ql = _dot_t(qb_s[h].astype(_bf16), w) * scale
                for b in range(_B):
                    qlat_s[b, pl.ds(h, 1), :] = ql[b:b + 1, :]
        _loop(part * 4, part * 4 + 4, body)

    def b_chunk(b, w):
        ck = ckv_v[w, pl.ds(4 * b, 4)].reshape(_WK, _DC)
        s = _dot_t(qlat_s[b].astype(_bf16), ck)
        m_old = m_s[b]
        m_new = jnp.maximum(m_old, jnp.max(s, axis=-1, keepdims=True))
        p = jnp.exp(s - m_new)
        alpha = jnp.exp(m_old - m_new)
        m_s[b] = m_new
        l_s[b] = alpha * l_s[b] + jnp.sum(p, axis=-1, keepdims=True)
        acc_s[b] = alpha * acc_s[b] + _dot(p.astype(_bf16), ck)

    def compute_ctx(part):
        def body(i):
            for j, w in enumerate(head_pair(i)):
                h = 2 * i + j
                lhs = two_rows(acc_s[0, pl.ds(h, 1), :], acc_s[1, pl.ds(h, 1), :])
                ctx_s[h] = _dot(lhs.astype(_bf16), w)
        _loop(part * 4, part * 4 + 4, body)

    def gated(q, h):
        gate = gate_s[...]
        return ((o_s[h] * gate) if q == 0 else (ctx_s[h] * (1.0 - gate))).astype(_bf16)

    def project(lhs, e, q, j6, j7):
        return _dot(lhs, wob_v[e, q, j7, pl.ds(j6 * _DH, _DH), :])

    def run(kv_sem, wq_sem, bw_sem, c_sem, e_sem, x_sem):
        def issue_region(src, block, dst, sem, w, unit, plan):
            for u in range(8):
                rows = _ds((w * 8 + u) * unit, unit)
                drows = pl.ds(u * unit, unit)
                for step in plan:
                    for q, (j, half) in enumerate(step):
                        if half is None:
                            _start(src.at[block(j), :, rows], dst.at[j, :, drows], sem, q)
                        else:
                            _start(src.at[pl.ds(block(j), 2), half, rows], dst.at[pl.ds(j, 2), half, drows], sem, q)

        def issue_kv(src, n, last):
            slot = n % _NSLOT
            if last:
                block, plan = (lambda j: ((_NG - 1) * 8 + _ROT + j) % (_B * _H)), (_PLAN_WRAP if _ROT else _PLAN)
            else:
                first = jnp.minimum(n // (2 * _NW), _NG - 2) * 8 + _ROT
                block, plan = (lambda j: first + j), _PLAN
            issue_region(src, block, kv_buf.at[slot], kv_sem.at[slot], n % _NW, 64, plan)

        def wq_piece(x):
            idx = (slice(None), _ds((x // 4) * 8, 8), _ds((x % 4) * 1024, 1024))
            return wq_hbm.at[idx], wq_v.at[idx], wq_sem

        def bw_piece(j):
            src = (bwq_hbm, bwuk_hbm, bwuv_hbm)[j]
            return lambda x: (src.at[:, _ds(x * 64, 64)], bw_v.at[j, :, _ds(x * 64, 64)], bw_sem)

        def issue_weights(w):
            for u in range(8):
                for pieces in ((wq_piece, bw_piece(1)), (bw_piece(0), bw_piece(2))):
                    for j6 in range(2):
                        for q in range(2):
                            _start(*pieces[q](j6 * 64 + w * 8 + u), q)

        def end_piece(e, q, j6, u):
            return ((wo_hbm, bwo_hbm)[q].at[:, _ds(j6 * 1024 + e * 128 + u * 16, 16)],
                    wob_v.at[e, q, :, pl.ds(j6 * 128 + u * 16, 16)])

        def issue_end(chunks):
            for u in range(8):
                for e in chunks:
                    for j6 in range(2):
                        for q in range(2):
                            _start(*end_piece(e, q, j6, u), e_sem.at[e], q)

        def weights_step(w):
            issue_weights(w)

            @pl.when(w == 0)
            def _():
                _start(x_hbm, x_ref, x_sem.at[0], 0)
                _start(gw_hbm, gw_ref, x_sem.at[1], 0)
        _loop(0, _NW, weights_step)

        o_s[...] = jnp.zeros_like(o_s)
        m_s[...] = jnp.full_like(m_s, -jnp.inf)
        l_s[...] = jnp.zeros_like(l_s)
        acc_s[...] = jnp.zeros_like(acc_s)
        reset_group()
        _wait_all(x_ref, x_sem.at[0])
        _wait_all(gw_ref, x_sem.at[1])
        xf = x_ref[...].astype(_f32)
        x8 = two_rows(xf[0:1], xf[1:2])
        x_s[...] = x8
        gate = jax.nn.sigmoid(jnp.sum(x8 * gw_ref[...].astype(_f32).reshape(1, _D), axis=-1, keepdims=True))
        gate_s[...] = jnp.broadcast_to(gate, (8, _DH))

        _loop(0, _NW, lambda w: issue_region(ckv_hbm, lambda j: j, ckv_v.at[w], c_sem, w, 16, _PLAN_CKV))
        _wait_all(wq_v, wq_sem)
        compute_qa()

        nkv = _NG * 2 * _NW

        def step(t):
            is_v = (t // _NW) % 2 == 1
            last = t >= nkv - 2 * _NW
            for src, want_v in ((k_hbm, False), (v_hbm, True)):
                @pl.when((is_v == want_v) & jnp.logical_not(last))
                def _():
                    issue_kv(src, t, False)

                @pl.when((is_v == want_v) & last & (t < nkv))
                def _():
                    issue_kv(src, t, True)

            @pl.when(t >= nkv)
            def _():
                e = jnp.maximum(t - nkv, 0)
                issue_end((e, e + 4))

            @pl.when(t >= _LAG)
            def _():
                n = jnp.maximum(t - _LAG, 0)
                slot = n % _NSLOT
                g = n // (2 * _NW)
                w = n % _NW
                _wait_all(kv_buf.at[slot], kv_sem.at[slot])
                pl.when((n // _NW) % 2 == 0)(lambda: k_window(g, w, slot))
                pl.when((n // _NW) % 2 == 1)(lambda: v_window(w, slot))

                @pl.when(n % (2 * _NW) == 2 * _NW - 1)
                def _():
                    finish_group(g)
                    reset_group()

            first = 0

            def tasks(count, fn):
                nonlocal first
                lo = first
                first += count
                pl.when((t >= lo) & (t < lo + count))(lambda: fn(jnp.clip(t - lo, 0, count - 1)))

            def normalize(_):
                acc_s[...] = acc_s[...] / l_s[...]

            tasks(1, lambda _: _wait_all(bw_v, bw_sem))
            tasks(2, lambda i: to_words(0, i))
            tasks(4, compute_qb)
            tasks(2, lambda i: to_words(1, i))
            tasks(4, compute_qlat)
            tasks(1, lambda _: _wait_all(ckv_v, c_sem))
            tasks(_B * _NW, lambda i: b_chunk(i % _B, i // _B))
            tasks(1, normalize)
            tasks(2, lambda i: to_words(2, i))
            tasks(4, compute_ctx)
        _loop(0, nkv + _LAG, step)

        parts = (((0, 0), (1, 0)), ((0, 1),), ((1, 1),))
        views = (wob_v.at[7, :, :, pl.ds(0, _DH)], wob_v.at[7, 0, :, pl.ds(_DH, _DH)],
                 wob_v.at[7, 1, :, pl.ds(_DH, _DH)])
        issue_end((3,))
        for i, part in enumerate(parts):
            for u in range(8):
                for k, (q, j6) in enumerate(part):
                    _start(*end_piece(7, q, j6, u), e_sem.at[7 + i], (u * len(part) + k) % 2)

        def chunk(i, acc):
            e = i // 2 + (i % 2) * 4
            _wait_all(wob_v.at[e], e_sem.at[e])
            for q in range(2):
                for j in range(4):
                    acc = acc + project(gated(q, e + 8 * j), e, q, j % 2, j // 2)
            return acc
        res = jax.lax.fori_loop(0, 7, chunk, jnp.zeros((8, _D), _f32))
        for i, part in enumerate(parts):
            blocks = [(q, j6, j7) for q, j6 in part for j7 in range(2)]
            left = [gated(q, 7 + 8 * j6 + 16 * j7) for q, j6, j7 in blocks]
            _wait_all(views[i], e_sem.at[7 + i])
            for blk, lhs in zip(blocks, left):
                res = res + project(lhs, 7, *blk)
        out_ref[...] = res[0:2, :].astype(_bf16)

    dma = pltpu.SemaphoreType.DMA
    pl.run_scoped(run, dma((_NSLOT,)), dma(()), dma(()), dma(()), dma((10,)), dma((2,)))


@jax.jit
def pallas_gated_mix__mha_block_cached__compressed_kv_cla__decode_kernel(
    A_x: jax.Array,
    A_k_cache: jax.Array,
    A_v_cache: jax.Array,
    A_wq: jax.Array,
    A_wo: jax.Array,
    B_x: jax.Array,
    B_c_kv: jax.Array,
    B_w_q: jax.Array,
    B_w_uk: jax.Array,
    B_w_uv: jax.Array,
    B_w_o: jax.Array,
    gate_w: jax.Array,
):
    del B_x
    k4 = A_k_cache.reshape(_B * _H, 2, _SK // 2, _DH)
    v4 = A_v_cache.reshape(_B * _H, 2, _SK // 2, _DH)
    ckv = B_c_kv.reshape(8, 2, _SK // 8, _DC)
    wq = A_wq.reshape(2, _D // 2, _H * _DH)
    bwq = B_w_q.reshape(2, _D * _H // 2, _DH)
    bwuk = B_w_uk.reshape(2, _DC * _H // 2, _DH)
    bwuv = B_w_uv.reshape(2, _DC * _H // 2, _DH)
    wo = A_wo.reshape(2, _H * _DH // 2, _D)
    bwo = B_w_o.reshape(2, _H * _DH // 2, _D)
    x2 = A_x.reshape(_B, _D)

    hbm = pl.BlockSpec(memory_space=pl.ANY)
    vmem = pl.BlockSpec(memory_space=pltpu.VMEM)
    V = pltpu.VMEM
    scratch = [
        V((_NSLOT, 8, 2, _WK // 2, _DH), _bf16),
        V((2, _D // 2, _H * _DH), _bf16),
        V((8, 2, 2, 2 * _DH, _D), _bf16),
        V((_NW, 8, 2, _WK // 8, _DC), _bf16),
        V((3, 2, _D * _H // 2, _DH), _bf16),
        V((_D * _H // 2, _DH), jnp.int32),
        V((8, _D), _f32),
        V((8, _DH), _f32),
        V((_B * _H, _DH), _f32),
        V((_H, 8, _DH), _f32),
        V((_B, _H, _DC), _f32),
        V((_H, 8, _DH), _f32),
        V((_H, 8, _DH), _f32),
        V((8, _SK), _f32),
        V((8, _DH), _f32),
        V((8, _DH), _f32),
        V((8, _DH), _f32),
        V((_B, _H, 1), _f32),
        V((_B, _H, 1), _f32),
        V((_B, _H, _DC), _f32),
        V((_B, _D), _bf16),
        V((_D,), _bf16),
    ]
    out = pl.pallas_call(
        _kernel,
        out_shape=jax.ShapeDtypeStruct((_B, _D), _bf16),
        in_specs=[hbm] * 11,
        out_specs=vmem,
        scratch_shapes=scratch,
        compiler_params=pltpu.CompilerParams(vmem_limit_bytes=100 * 1024 * 1024),
    )(x2, gate_w, k4, v4, wq, wo, ckv, bwq, bwuk, bwuv, bwo)
    return out.reshape(_B, 1, _D)
```

```python
import jax
import jax.numpy as jnp
import jax.experimental.pallas as pl
import jax.experimental.pallas.tpu as pltpu

_B, _H, _SK, _DH, _D, _DC = 2, 32, 8192, 128, 512, 512

_NW = 8
_NG = _B * _H // 8
_WK = _SK // _NW
_LAG = 3
_NSLOT = _LAG + 1
_ROT = 1

_PLAN = (((0, 0), (4, 0)), ((0, 1), (4, 1)), ((2, 0), (6, 0)), ((2, 1), (6, 1)))
_PLAN_WRAP = (((0, 0), (7, None)), ((0, 1), (4, 1)), ((2, 0), (4, 0)), ((2, 1), (6, None)))
_PLAN_CKV = (((1, 0), (0, None)), ((1, 1), (5, 1)), ((3, 0), (5, 0)), ((3, 1), (7, None)))

_PP = 2
_BS = 2

_f32 = jnp.float32
_bf16 = jnp.bfloat16


def _dot(a, b):
    return jnp.dot(a, b, preferred_element_type=_f32)


def _dot_t(a, b):
    return jax.lax.dot_general(a, b, (((1,), (1,)), ((), ())), preferred_element_type=_f32)


def _unpack_pair(blk):
    lo = pltpu.bitcast(blk << 16, _f32).astype(_bf16)
    hi = pltpu.bitcast(blk & jnp.int32(-65536), _f32).astype(_bf16)
    return lo, hi


def _fold(x, op):
    parts = [x[:, i:i + 128] for i in range(0, x.shape[1], 128)]
    while len(parts) > 1:
        parts = [op(parts[i], parts[i + 1]) for i in range(0, len(parts), 2)]
    return parts[0]


def _ds(first, size):
    return pl.ds(first if isinstance(first, int) else pl.multiple_of(first, size), size)


def _loop(lo, hi, body):
    jax.lax.fori_loop(lo, hi, lambda i, c: (body(i), c)[1], 0)


def _start(src, dst, sem, prio):
    pltpu.make_async_copy(src, dst, sem).start(priority=prio)


def _wait_all(dst, sem):
    pltpu.make_async_copy(dst, dst, sem).wait()


def _kernel(x_hbm, gw_hbm, k_hbm, v_hbm, wq_hbm, wo_hbm, ckv_hbm, bwq_hbm, bwuk_hbm, bwuv_hbm, bwo_hbm,
            out_ref,
            kv_buf, wq_v, wob_v, ckv_v, bw_v, w32,
            x_s, gate_s, qa_s, qb_s, qlat_s, o_s, ctx_s, s_s, mv_s, lv_s, av_s, m_s, l_s, acc_s,
            x_ref, gw_ref):
    row8 = jax.lax.broadcasted_iota(jnp.int32, (8, _D), 0)
    row8h = jax.lax.broadcasted_iota(jnp.int32, (8, _DH), 0)
    row8k = jax.lax.broadcasted_iota(jnp.int32, (8, _WK), 0)
    scale = _DH ** -0.5

    def two_rows(r0, r1):
        return jnp.where(row8 == 0, r0, jnp.where(row8 == 1, r1, 0.0))

    def compute_qa():
        def body(c):
            q = _dot(x_s[...].astype(_bf16), wq_v[:, :, _ds(c * 512, 512)].reshape(_D, 512)) * scale
            for j in range(4):
                for b in range(_B):
                    row = (b * _H + 4 * c + j + _B * _H - _ROT) % (_B * _H)
                    qa_s[pl.ds(row, 1), :] = q[b:b + 1, j * _DH:(j + 1) * _DH]
        _loop(0, _H // 4, body)

    def k_window(g, w, slot):
        q8 = qa_s[_ds(g * 8, 8), :].astype(_bf16)
        s = None
        for j in range(8):
            sj = _dot_t(q8, kv_buf[slot, j].reshape(_WK, _DH))
            s = sj if s is None else jnp.where(row8k == j, sj, s)
        s_s[:, _ds(w * _WK, _WK)] = s
        mv_s[...] = jnp.maximum(mv_s[...], _fold(s, jnp.maximum))

    def v_window(w, slot):
        m = jnp.max(mv_s[...], axis=-1, keepdims=True)
        p = jnp.exp(s_s[:, _ds(w * _WK, _WK)] - m)
        lv_s[...] += _fold(p, jnp.add)
        p = p.astype(_bf16)
        o = None
        for j in range(8):
            oj = _dot(p, kv_buf[slot, j].reshape(_WK, _DH))
            o = oj if o is None else jnp.where(row8h == j, oj, o)
        av_s[...] += o

    def reset_group():
        mv_s[...] = jnp.full_like(mv_s, -jnp.inf)
        lv_s[...] = jnp.zeros_like(lv_s)
        av_s[...] = jnp.zeros_like(av_s)

    def finish_group(g):
        o = av_s[...] / jnp.sum(lv_s[...], axis=-1, keepdims=True)
        for j in range(8):
            f = (g * 8 + j + _ROT) % (_B * _H)
            o_s[f % _H, pl.ds(f // _H, 1), :] = o[j:j + 1, :]

    def to_words(j, half):
        R = 256
        n = w32.shape[0] // (2 * R)
        def body(i):
            w32[_ds((half * n + i) * R, R), :] = pltpu.bitcast(bw_v[j, half, _ds(i * 2 * R, 2 * R), :], jnp.int32)
        _loop(0, n, body)

    def head_pair(i):
        return _unpack_pair(w32[pl.ds(i, _D, stride=_H // 2), :])

    def compute_qb(part):
        def body(i):
            for j, w in enumerate(head_pair(i)):
                qb_s[2 * i + j] = _dot(x_s[...].astype(_bf16), w)
        _loop(part * _PP, (part + 1) * _PP, body)

    def compute_qlat(part):
        def body(i):
            for j, w in enumerate(head_pair(i)):
                h = 2 * i + j
                ql = _dot_t(qb_s[h].astype(_bf16), w) * scale
                for b in range(_B):
                    qlat_s[b, pl.ds(h, 1), :] = ql[b:b + 1, :]
        _loop(part * _PP, (part + 1) * _PP, body)

    def b_chunk(i):
        nb = 4 // _BS
        w, b, part = i // (_B * _BS), i % _B, (i // _B) % _BS
        ck = ckv_v[w, pl.ds(4 * b + nb * part, nb)].reshape(_WK // _BS, _DC)
        s = _dot_t(qlat_s[b].astype(_bf16), ck)
        m_old = m_s[b]
        m_new = jnp.maximum(m_old, jnp.max(s, axis=-1, keepdims=True))
        p = jnp.exp(s - m_new)
        alpha = jnp.exp(m_old - m_new)
        m_s[b] = m_new
        l_s[b] = alpha * l_s[b] + jnp.sum(p, axis=-1, keepdims=True)
        acc_s[b] = alpha * acc_s[b] + _dot(p.astype(_bf16), ck)

    def compute_ctx(part):
        def body(i):
            for j, w in enumerate(head_pair(i)):
                h = 2 * i + j
                lhs = two_rows(acc_s[0, pl.ds(h, 1), :], acc_s[1, pl.ds(h, 1), :])
                ctx_s[h] = _dot(lhs.astype(_bf16), w)
        _loop(part * _PP, (part + 1) * _PP, body)

    def gated(q, h):
        gate = gate_s[...]
        return ((o_s[h] * gate) if q == 0 else (ctx_s[h] * (1.0 - gate))).astype(_bf16)

    def project(lhs, e, q, j6, j7):
        return _dot(lhs, wob_v[e, q, j7, pl.ds(j6 * _DH, _DH), :])

    def run(kv_sem, wq_sem, bw_sem, c_sem, e_sem, x_sem):
        def issue_region(src, block, dst, sem, w, unit, plan):
            for u in range(8):
                rows = _ds((w * 8 + u) * unit, unit)
                drows = pl.ds(u * unit, unit)
                for step in plan:
                    for q, (j, half) in enumerate(step):
                        if half is None:
                            _start(src.at[block(j), :, rows], dst.at[j, :, drows], sem, q)
                        else:
                            _start(src.at[pl.ds(block(j), 2), half, rows], dst.at[pl.ds(j, 2), half, drows], sem, q)

        def issue_kv(src, n, last):
            slot = n % _NSLOT
            if last:
                block, plan = (lambda j: ((_NG - 1) * 8 + _ROT + j) % (_B * _H)), (_PLAN_WRAP if _ROT else _PLAN)
            else:
                first = jnp.minimum(n // (2 * _NW), _NG - 2) * 8 + _ROT
                block, plan = (lambda j: first + j), _PLAN
            issue_region(src, block, kv_buf.at[slot], kv_sem.at[slot], n % _NW, 64, plan)

        def wq_piece(x):
            idx = (slice(None), _ds((x // 4) * 8, 8), _ds((x % 4) * 1024, 1024))
            return wq_hbm.at[idx], wq_v.at[idx], wq_sem

        def bw_piece(j):
            src = (bwq_hbm, bwuk_hbm, bwuv_hbm)[j]
            return lambda x: (src.at[:, _ds(x * 64, 64)], bw_v.at[j, :, _ds(x * 64, 64)], bw_sem)

        def issue_weights(w):
            for u in range(8):
                for pieces in ((wq_piece, bw_piece(1)), (bw_piece(0), bw_piece(2))):
                    for j6 in range(2):
                        for q in range(2):
                            _start(*pieces[q](j6 * 64 + w * 8 + u), q)

        def end_piece(e, q, j6, u):
            return ((wo_hbm, bwo_hbm)[q].at[:, _ds(j6 * 1024 + e * 128 + u * 16, 16)],
                    wob_v.at[e, q, :, pl.ds(j6 * 128 + u * 16, 16)])

        def issue_end(chunks):
            for u in range(8):
                for e in chunks:
                    for j6 in range(2):
                        for q in range(2):
                            _start(*end_piece(e, q, j6, u), e_sem.at[e], q)

        def weights_step(w):
            issue_weights(w)

            @pl.when(w == 0)
            def _():
                _start(x_hbm, x_ref, x_sem.at[0], 0)
                _start(gw_hbm, gw_ref, x_sem.at[1], 0)
        _loop(0, _NW, weights_step)

        o_s[...] = jnp.zeros_like(o_s)
        m_s[...] = jnp.full_like(m_s, -jnp.inf)
        l_s[...] = jnp.zeros_like(l_s)
        acc_s[...] = jnp.zeros_like(acc_s)
        reset_group()
        _wait_all(x_ref, x_sem.at[0])
        _wait_all(gw_ref, x_sem.at[1])
        xf = x_ref[...].astype(_f32)
        x8 = two_rows(xf[0:1], xf[1:2])
        x_s[...] = x8
        gate = jax.nn.sigmoid(jnp.sum(x8 * gw_ref[...].astype(_f32).reshape(1, _D), axis=-1, keepdims=True))
        gate_s[...] = jnp.broadcast_to(gate, (8, _DH))

        _loop(0, _NW, lambda w: issue_region(ckv_hbm, lambda j: j, ckv_v.at[w], c_sem, w, 16, _PLAN_CKV))
        _wait_all(wq_v, wq_sem)
        compute_qa()

        nkv = _NG * 2 * _NW

        def step(t):
            is_v = (t // _NW) % 2 == 1
            last = t >= nkv - 2 * _NW
            for src, want_v in ((k_hbm, False), (v_hbm, True)):
                @pl.when((is_v == want_v) & jnp.logical_not(last))
                def _():
                    issue_kv(src, t, False)

                @pl.when((is_v == want_v) & last & (t < nkv))
                def _():
                    issue_kv(src, t, True)

            @pl.when(t >= nkv)
            def _():
                e = jnp.maximum(t - nkv, 0)
                issue_end((e, e + 4))

            @pl.when(t >= _LAG)
            def _():
                n = jnp.maximum(t - _LAG, 0)
                slot = n % _NSLOT
                g = n // (2 * _NW)
                w = n % _NW
                _wait_all(kv_buf.at[slot], kv_sem.at[slot])
                pl.when((n // _NW) % 2 == 0)(lambda: k_window(g, w, slot))
                pl.when((n // _NW) % 2 == 1)(lambda: v_window(w, slot))

                @pl.when(n % (2 * _NW) == 2 * _NW - 1)
                def _():
                    finish_group(g)
                    reset_group()

            first = 0

            def tasks(count, fn):
                nonlocal first
                lo = first
                first += count
                pl.when((t >= lo) & (t < lo + count))(lambda: fn(jnp.clip(t - lo, 0, count - 1)))

            def normalize(_):
                acc_s[...] = acc_s[...] / l_s[...]

            tasks(1, lambda _: _wait_all(bw_v, bw_sem))
            tasks(2, lambda i: to_words(0, i))
            tasks(_H // 2 // _PP, compute_qb)
            tasks(2, lambda i: to_words(1, i))
            tasks(_H // 2 // _PP, compute_qlat)
            tasks(1, lambda _: _wait_all(ckv_v, c_sem))
            tasks(_B * _NW * _BS, b_chunk)
            tasks(1, normalize)
            tasks(2, lambda i: to_words(2, i))
            tasks(_H // 2 // _PP, compute_ctx)
        _loop(0, nkv + _LAG, step)

        parts = (((0, 0), (1, 0)), ((0, 1),), ((1, 1),))
        views = (wob_v.at[7, :, :, pl.ds(0, _DH)], wob_v.at[7, 0, :, pl.ds(_DH, _DH)],
                 wob_v.at[7, 1, :, pl.ds(_DH, _DH)])
        issue_end((3,))
        for i, part in enumerate(parts):
            for u in range(8):
                for k, (q, j6) in enumerate(part):
                    _start(*end_piece(7, q, j6, u), e_sem.at[7 + i], (u * len(part) + k) % 2)

        def chunk(i, acc):
            e = i // 2 + (i % 2) * 4
            _wait_all(wob_v.at[e], e_sem.at[e])
            for q in range(2):
                for j in range(4):
                    acc = acc + project(gated(q, e + 8 * j), e, q, j % 2, j // 2)
            return acc
        res = jax.lax.fori_loop(0, 7, chunk, jnp.zeros((8, _D), _f32))
        for i, part in enumerate(parts):
            blocks = [(q, j6, j7) for q, j6 in part for j7 in range(2)]
            left = [gated(q, 7 + 8 * j6 + 16 * j7) for q, j6, j7 in blocks]
            _wait_all(views[i], e_sem.at[7 + i])
            for blk, lhs in zip(blocks, left):
                res = res + project(lhs, 7, *blk)
        out_ref[...] = res[0:2, :].astype(_bf16)

    dma = pltpu.SemaphoreType.DMA
    pl.run_scoped(run, dma((_NSLOT,)), dma(()), dma(()), dma(()), dma((10,)), dma((2,)))


@jax.jit
def pallas_gated_mix__mha_block_cached__compressed_kv_cla__decode_kernel(
    A_x: jax.Array,
    A_k_cache: jax.Array,
    A_v_cache: jax.Array,
    A_wq: jax.Array,
    A_wo: jax.Array,
    B_x: jax.Array,
    B_c_kv: jax.Array,
    B_w_q: jax.Array,
    B_w_uk: jax.Array,
    B_w_uv: jax.Array,
    B_w_o: jax.Array,
    gate_w: jax.Array,
):
    del B_x
    k4 = A_k_cache.reshape(_B * _H, 2, _SK // 2, _DH)
    v4 = A_v_cache.reshape(_B * _H, 2, _SK // 2, _DH)
    ckv = B_c_kv.reshape(8, 2, _SK // 8, _DC)
    wq = A_wq.reshape(2, _D // 2, _H * _DH)
    bwq = B_w_q.reshape(2, _D * _H // 2, _DH)
    bwuk = B_w_uk.reshape(2, _DC * _H // 2, _DH)
    bwuv = B_w_uv.reshape(2, _DC * _H // 2, _DH)
    wo = A_wo.reshape(2, _H * _DH // 2, _D)
    bwo = B_w_o.reshape(2, _H * _DH // 2, _D)
    x2 = A_x.reshape(_B, _D)

    hbm = pl.BlockSpec(memory_space=pl.ANY)
    vmem = pl.BlockSpec(memory_space=pltpu.VMEM)
    V = pltpu.VMEM
    scratch = [
        V((_NSLOT, 8, 2, _WK // 2, _DH), _bf16),
        V((2, _D // 2, _H * _DH), _bf16),
        V((8, 2, 2, 2 * _DH, _D), _bf16),
        V((_NW, 8, 2, _WK // 8, _DC), _bf16),
        V((3, 2, _D * _H // 2, _DH), _bf16),
        V((_D * _H // 2, _DH), jnp.int32),
        V((8, _D), _f32),
        V((8, _DH), _f32),
        V((_B * _H, _DH), _f32),
        V((_H, 8, _DH), _f32),
        V((_B, _H, _DC), _f32),
        V((_H, 8, _DH), _f32),
        V((_H, 8, _DH), _f32),
        V((8, _SK), _f32),
        V((8, _DH), _f32),
        V((8, _DH), _f32),
        V((8, _DH), _f32),
        V((_B, _H, 1), _f32),
        V((_B, _H, 1), _f32),
        V((_B, _H, _DC), _f32),
        V((_B, _D), _bf16),
        V((_D,), _bf16),
    ]
    out = pl.pallas_call(
        _kernel,
        out_shape=jax.ShapeDtypeStruct((_B, _D), _bf16),
        in_specs=[hbm] * 11,
        out_specs=vmem,
        scratch_shapes=scratch,
        compiler_params=pltpu.CompilerParams(vmem_limit_bytes=100 * 1024 * 1024),
    )(x2, gate_w, k4, v4, wq, wo, ckv, bwq, bwuk, bwuv, bwo)
    return out.reshape(_B, 1, _D)
```
